```python
import jax
import jax.numpy as jnp

def _softmax(x, axis=-1):
    return jax.nn.softmax(x, axis=axis)
def _gelu(x):
    return jax.nn.gelu(x, approximate=True)
def _silu(x):
    return jax.nn.silu(x)
def _sigmoid(x):
    return jax.nn.sigmoid(x)
def _layernorm(x, axis=-1, eps=1e-5):
    m = jnp.mean(x, axis=axis, keepdims=True)
    v = jnp.var(x, axis=axis, keepdims=True)
    return (x - m) / jnp.sqrt(v + eps)
def _scatter_add(tgt, idx, src, axis=0):
    return tgt.at[idx].add(src)
def _segment_sum(src, seg, n):
    return jax.ops.segment_sum(src, seg, n)
class _Rng:
    def __init__(self, key):
        self._k = key
    def _next(self):
        self._k, sub = jax.random.split(self._k)
        return sub
    def normal(self, shape):
        return jax.random.normal(self._next(), shape, dtype=jnp.bfloat16)
    def randint(self, lo, hi, shape):
        return jax.random.randint(self._next(), shape, lo, hi, dtype=jnp.int32)
    def uniform(self, shape, lo=0.0, hi=1.0):
        return jax.random.uniform(self._next(), shape, jnp.bfloat16, lo, hi)
    def permutation(self, n):
        return jax.random.permutation(self._next(), n)


kernel_name = 'concat_heads__compressed_kv_cla__mha_block_cached__decode'

def setup_inputs():
    _rng = _Rng(jax.random.key(int.from_bytes(__import__("os").urandom(4), "little")))
    _w = (lambda a: (lambda t: t.astype(jnp.bfloat16) if jnp.issubdtype(t.dtype, jnp.floating) else t)(jnp.asarray(a)))
    def _A_setup():
        B, H, Sq, Sk, D, M = 4, 32, 1, 4096, 128, 512
        Dc = 4 * D
        return {
            "x": _w((lambda *s: _rng.normal(s) * 0.05)(B, Sq, M)),
            "c_kv": _w((lambda *s: _rng.normal(s) * 0.05)(B, Sk, Dc)),
            "w_q": _w((lambda *s: _rng.normal(s) * 0.05)(M, H, D) * (M ** -0.5)),
            "w_uk": _w((lambda *s: _rng.normal(s) * 0.05)(Dc, H, D) * (Dc ** -0.5)),
            "w_uv": _w((lambda *s: _rng.normal(s) * 0.05)(Dc, H, D) * (Dc ** -0.5)),
            "w_o": _w((lambda *s: _rng.normal(s) * 0.05)(H, D, M) * ((H * D) ** -0.5)),
        }
    _A_in = _A_setup()

    def _B_setup():
        B, Sq, D = 4, 1, 512
        H, Sk, Dh = 32, 4096, 128
        return {
            "x": _w((lambda *s: _rng.normal(s) * 0.05)(B, Sq, D)),
            "k_cache": _w((lambda *s: _rng.normal(s) * 0.05)(B, H, Sk, Dh)),
            "v_cache": _w((lambda *s: _rng.normal(s) * 0.05)(B, H, Sk, Dh)),
            "wq": _w((lambda *s: _rng.normal(s) * 0.05)(D, H * Dh) * (D ** -0.5)),
            "wo": _w((lambda *s: _rng.normal(s) * 0.05)(H * Dh, D) * ((H * Dh) ** -0.5)),
        }
    _B_in = _B_setup()

    return {
        "A_x": _A_in["x"],
        "A_c_kv": _A_in["c_kv"],
        "A_w_q": _A_in["w_q"],
        "A_w_uk": _A_in["w_uk"],
        "A_w_uv": _A_in["w_uv"],
        "A_w_o": _A_in["w_o"],
        "B_x": _B_in["x"],
        "B_k_cache": _B_in["k_cache"],
        "B_v_cache": _B_in["v_cache"],
        "B_wq": _B_in["wq"],
        "B_wo": _B_in["wo"],
    }

def reference(A_x, A_c_kv, A_w_q, A_w_uk, A_w_uv, A_w_o, B_x, B_k_cache, B_v_cache, B_wq, B_wo):
    def _A_ref(x, c_kv, w_q, w_uk, w_uv, w_o):
        B, Sq, M = x.shape[0], x.shape[1], x.shape[2]
        Sk = c_kv.shape[1]
        H, D = w_q.shape[1], w_q.shape[2]
        q = jnp.einsum("bqm,mhd->bhqd", x, w_q)
        k = jnp.einsum("bkc,chd->bhkd", c_kv, w_uk)
        v = jnp.einsum("bkc,chd->bhkd", c_kv, w_uv)
        scores = jnp.einsum("bhqd,bhkd->bhqk", q, k) * (D ** -0.5)
        off = Sk - Sq
        qi = jnp.arange(Sq)[:, None]
        kj = jnp.arange(Sk)[None, :]
        cmask = kj <= (qi + off)
        scores = jnp.where(cmask[None, None], scores, -1e9)
        p = _softmax(scores, axis=-1)
        ctx = jnp.einsum("bhqk,bhkd->bhqd", p, v)
        return jnp.einsum("bhqd,hdm->bqm", ctx, w_o)

    def _B_ref(x, k_cache, v_cache, wq, wo):
        B, Sq, D = x.shape
        H, Dh = 32, 128
        q = (lambda x, *d: x.transpose(*d))((x @ wq).reshape(B, Sq, H, Dh), 0, 2, 1, 3)
        scores = jnp.einsum("bhqd,bhkd->bhqk", q, k_cache) * (Dh ** -0.5)
        p = _softmax(scores, axis=-1)
        o = jnp.einsum("bhqk,bhkd->bhqd", p, v_cache)
        return (lambda x, *d: x.transpose(*d))(o, 0, 2, 1, 3).reshape(B, Sq, H * Dh) @ wo

    a = _A_ref(A_x, A_c_kv, A_w_q, A_w_uk, A_w_uv, A_w_o)
    b = _B_ref(B_x, B_k_cache, B_v_cache, B_wq, B_wo)
    return jnp.concatenate([a, b], axis=-1)
```

```python
import jax
import jax.numpy as jnp
import numpy as np
import jax.experimental.pallas as pl
import jax.experimental.pallas.tpu as pltpu

B, H, SK, D, M, DC = 4, 32, 4096, 128, 512, 512
T = 128
NJ = SK // T
NP = 2 * B
NT = (((1,), (1,)), ((), ()))
F32, BF16 = jnp.float32, jnp.bfloat16


def build(nbuf=2, S=1, rows=64, hmajor=False, prio=1, xrows=64, nochk=True):
    xe = xrows * 128

    def kernel(ax_h, ckv_h, awq_h, wuk_h, wuv_h, awo_h, bx_h, k_h, v_h, bwq_h, bwo_h,
               out_ref,
               ax_v, bx_v, ckv_v, awq_v, wuk_v, wuv_v, awo_v, bwq_v, bwo_v, ring,
               qb_s, s_s, p_s, oacc_s, ob_s, qabs_s, sa_s, pa_s, cacc_s, ctxc_s, ctx_s, outa_s,
               ring_sem, w_sem, x_sem):
        sub8 = jax.lax.broadcasted_iota(jnp.int32, (8, 128), 0)

        u32 = lambda r: r.bitcast(jnp.uint32)
        side = [[(u32(awq_h), awq_v, 0), (u32(wuk_h), wuk_v, 1)]]
        side += [[(ckv_h.at[b], ckv_v.at[b], 2 + b)] for b in range(B)]
        side += [[(u32(wuv_h), wuv_v, 6)], [(awo_h, awo_v, 7)], [(bwo_h, bwo_v, 8)]]

        def side_pieces(src, dst, sem_i, j, nj):
            r, c = src.shape
            pack = 4 // src.dtype.itemsize
            ne = xe * pack // 2
            pr = max(8 * pack, ne // c)
            pc = min(c, ne // pr)
            per_r = r // nj
            out = []
            for r0 in range(0, per_r, pr):
                for c0 in range(0, c, pc):
                    idx = (pl.ds(j * per_r + r0, pr), pl.ds(c0, pc))
                    out.append(pltpu.make_async_copy(src.at[idx], dst.at[idx], w_sem.at[sem_i]))
            return out

        def start_all(copies):
            for n, cp in enumerate(copies):
                cp.start(priority=(n % 2) if prio else 0)

        def issue(p, j, slot):
            src = (k_h if p % 2 == 0 else v_h).at[p // 2]
            hs, rs = range(0, H, S), range(0, T, rows)
            order = [(h, r) for h in hs for r in rs] if hmajor else [(h, r) for r in rs for h in hs]
            main = [pltpu.make_async_copy(
                src.at[pl.ds(h, S), pl.ds(j * T + r, rows)],
                ring.at[slot, pl.ds(h, S), pl.ds(r, rows)], ring_sem.at[slot]) for h, r in order]
            extra = []
            for a in side[p]:
                extra += side_pieces(*a, j, NJ)
            start_all(main + extra)

        def issue_ahead(p, j, slot):
            if p + 1 < NP:
                @pl.when(j + nbuf < NJ)
                def _():
                    issue(p, j + nbuf, slot)

                @pl.when(j + nbuf >= NJ)
                def _():
                    issue(p + 1, j + nbuf - NJ, slot)
            else:
                @pl.when(j + nbuf < NJ)
                def _():
                    issue(p, j + nbuf, slot)

        def wait_ring(slot):
            pltpu.make_async_copy(ring.at[slot], ring.at[slot], ring_sem.at[slot]).wait()

        def wait_side(dst, sem_i):
            pltpu.make_async_copy(dst, dst, w_sem.at[sem_i]).wait()

        def bwq_issue(j, c):
            start_all(side_pieces(bwq_h, bwq_v, 9, j, NJ))
            return c
        cbx = pltpu.make_async_copy(bx_h, bx_v, x_sem.at[0])
        cax = pltpu.make_async_copy(ax_h, ax_v, x_sem.at[1])
        cbx.start()
        cax.start()
        jax.lax.fori_loop(0, NJ, bwq_issue, 0)
        for j in range(nbuf):
            issue(0, j, j)

        ob_s[...] = jnp.zeros_like(ob_s)
        ctxc_s[...] = jnp.zeros_like(ctxc_s)
        outa_s[...] = jnp.zeros_like(outa_s)
        cbx.wait()
        cax.wait()
        wait_side(bwq_v, 9)

        def pad8(x):
            return jnp.concatenate([x.astype(F32), jnp.zeros((8 - B, M), F32)], axis=0).astype(BF16)

        xb = pad8(bx_v[...])
        for h in range(H):
            r = jnp.dot(xb, bwq_v[:, h * D:(h + 1) * D], preferred_element_type=F32)
            qb_s[h * 8:(h + 1) * 8, :] = r

        def halves(ref, hp):
            u = ref[pl.ds(hp, M, stride=H // 2), :]
            lo = pltpu.bitcast(u << 16, F32).astype(BF16)
            hi = pltpu.bitcast(u & jnp.uint32(0xFFFF0000), F32).astype(BF16)
            return lo, hi

        def side_qabs(j):
            @pl.when(j % 2 == 0)
            def _():
                hp = j // 2
                xa = pad8(ax_v[...])
                wq = halves(awq_v, hp)
                wk = halves(wuk_v, hp)
                for e in range(2):
                    q = jnp.dot(xa, wq[e], preferred_element_type=F32).astype(BF16)
                    r = jax.lax.dot_general(q, wk[e], NT, preferred_element_type=F32)
                    row = pl.multiple_of((2 * hp + e) * 8, 8)
                    for c in range(DC // 128):
                        qabs_s[c, pl.ds(row, 8), :] = r[:, c * 128:(c + 1) * 128]

        AK = SK // (NJ // 2)

        def side_attn(b, j):
            @pl.when(j < NJ // 2)
            def _():
                q = jnp.concatenate(
                    [qabs_s[c, pl.ds(b, H, stride=8), :] for c in range(DC // 128)], axis=1).astype(BF16)
                c_blk = ckv_v[b, pl.ds(pl.multiple_of(j * AK, AK), AK), :]
                sa_s[j] = jax.lax.dot_general(q, c_blk, NT, preferred_element_type=F32) * (D ** -0.5)

            @pl.when(j == NJ // 2 - 1)
            def _():
                s = sa_s[...]
                m = jnp.max(jnp.max(s, axis=0), axis=1, keepdims=True)
                e = jnp.exp(s - m[None])
                l = jnp.sum(jnp.sum(e, axis=0), axis=1, keepdims=True)
                pa_s[...] = (e * (1.0 / l)[None]).astype(BF16)
                cacc_s[...] = jnp.zeros_like(cacc_s)

            @pl.when(j >= NJ // 2)
            def _():
                jj = j - NJ // 2
                c_blk = ckv_v[b, pl.ds(pl.multiple_of(jj * AK, AK), AK), :]
                cacc_s[...] += jnp.dot(pa_s[jj], c_blk, preferred_element_type=F32)

            @pl.when(j == NJ - 1)
            def _():
                for c in range(DC // 128):
                    ctxc_s[c, pl.ds(b, H, stride=8), :] = cacc_s[:, c * 128:(c + 1) * 128]

        def side_ctx(j):
            @pl.when(j % 2 == 0)
            def _():
                hp = j // 2
                wv = halves(wuv_v, hp)
                for e in range(2):
                    row = pl.multiple_of((2 * hp + e) * 8, 8)
                    lhs = jnp.concatenate(
                        [ctxc_s[c, pl.ds(row, 8), :] for c in range(DC // 128)], axis=1).astype(BF16)
                    ctx_s[pl.ds(row, 8), :] = jnp.dot(lhs, wv[e], preferred_element_type=F32)

        def side_outa(j):
            lhs = ctx_s[pl.ds(pl.multiple_of(j * 8, 8), 8), :].astype(BF16)
            w = awo_v[pl.ds(pl.multiple_of(j * D, D), D), :]
            outa_s[...] += jnp.dot(lhs, w, preferred_element_type=F32)

        side_compute = [None, side_qabs]
        side_compute += [(lambda j, b=b: side_attn(b, j)) for b in range(B)]
        side_compute += [side_ctx, side_outa]

        for p in range(NP):
            b = p // 2
            if p > 0:
                for _, dst, sem_i in side[p - 1]:
                    wait_side(dst, sem_i)
            if p % 2 == 1:
                s = s_s[...]
                m = jnp.max(jnp.max(s, axis=0), axis=1, keepdims=True)
                e = jnp.exp(s - m[None])
                l = jnp.sum(jnp.sum(e, axis=0), axis=1, keepdims=True)
                p_s[...] = e * (1.0 / l)[None]
                oacc_s[...] = jnp.zeros_like(oacc_s)

            def step(j, c, p=p, b=b):
                slot = j % nbuf
                wait_ring(slot)
                for g in range(H // 8):
                    if p % 2 == 0:
                        lhs = qb_s[pl.ds(g * 64 + b, 8, stride=8), :].astype(BF16)
                    else:
                        lhs = p_s[j, g * 8:(g + 1) * 8, :].astype(BF16)
                    acc = None
                    for hh in range(8):
                        t = ring[slot, g * 8 + hh]
                        if p % 2 == 0:
                            r = jax.lax.dot_general(lhs, t, NT, preferred_element_type=F32)
                        else:
                            r = jnp.dot(lhs, t, preferred_element_type=F32)
                        acc = r if acc is None else jnp.where(sub8 == hh, r, acc)
                    if p % 2 == 0:
                        s_s[j, g * 8:(g + 1) * 8, :] = acc * (D ** -0.5)
                    else:
                        oacc_s[g * 8:(g + 1) * 8, :] += acc
                issue_ahead(p, j, slot)
                if side_compute[p] is not None:
                    side_compute[p](j)
                return c

            jax.lax.fori_loop(0, NJ, step, 0)
            if p % 2 == 1:
                ob_s[pl.ds(b, H, stride=8), :] = oacc_s[...]

        wait_side(bwo_v, 8)
        outb = jnp.zeros((8, M), F32)
        for h in range(H):
            outb += jnp.dot(ob_s[h * 8:(h + 1) * 8, :].astype(BF16), bwo_v[h * D:(h + 1) * D, :],
                            preferred_element_type=F32)
        out_ref[:, 0:M] = outa_s[0:B, :].astype(out_ref.dtype)
        out_ref[:, M:2 * M] = outb[0:B, :].astype(out_ref.dtype)

    assert NJ % nbuf == 0
    hbm = pl.BlockSpec(memory_space=pltpu.HBM)
    AK = SK // (NJ // 2)

    def run(A_x, A_c_kv, A_w_q, A_w_uk, A_w_uv, A_w_o, B_x, B_k_cache, B_v_cache, B_wq, B_wo):
        out = pl.pallas_call(
            kernel,
            out_shape=jax.ShapeDtypeStruct((B, 2 * M), A_x.dtype),
            in_specs=[hbm] * 11,
            out_specs=pl.BlockSpec(memory_space=pltpu.VMEM),
            scratch_shapes=[
                pltpu.VMEM((B, M), BF16), pltpu.VMEM((B, M), BF16),
                pltpu.VMEM((B, SK, DC), BF16),
                pltpu.VMEM((M * H // 2, D), jnp.uint32), pltpu.VMEM((DC * H // 2, D), jnp.uint32), pltpu.VMEM((DC * H // 2, D), jnp.uint32),
                pltpu.VMEM((H * D, M), BF16), pltpu.VMEM((M, H * D), BF16), pltpu.VMEM((H * D, M), BF16),
                pltpu.VMEM((nbuf, H, T, D), BF16),
                pltpu.VMEM((H * 8, D), F32),
                pltpu.VMEM((NJ, H, T), F32),
                pltpu.VMEM((NJ, H, T), F32),
                pltpu.VMEM((H, D), F32),
                pltpu.VMEM((H * 8, D), F32),
                pltpu.VMEM((DC // 128, H * 8, 128), F32),
                pltpu.VMEM((NJ // 2, H, AK), F32),
                pltpu.VMEM((NJ // 2, H, AK), BF16),
                pltpu.VMEM((H, DC), F32),
                pltpu.VMEM((DC // 128, H * 8, 128), F32),
                pltpu.VMEM((H * 8, D), F32),
                pltpu.VMEM((8, M), F32),
                pltpu.SemaphoreType.DMA((nbuf,)),
                pltpu.SemaphoreType.DMA((10,)),
                pltpu.SemaphoreType.DMA((2,)),
            ],
            compiler_params=pltpu.CompilerParams(
                vmem_limit_bytes=100 * 1024 * 1024, disable_bounds_checks=nochk),
        )(A_x.reshape(B, M), A_c_kv, A_w_q.reshape(M * H, D), A_w_uk.reshape(DC * H, D),
          A_w_uv.reshape(DC * H, D), A_w_o.reshape(H * D, M), B_x.reshape(B, M),
          B_k_cache, B_v_cache, B_wq, B_wo)
        return out.reshape(B, 1, 2 * M)

    return run


_run = build()


@jax.jit
def pallas_concat_heads__compressed_kv_cla__mha_block_cached__decode_kernel(
    A_x, A_c_kv, A_w_q, A_w_uk, A_w_uv, A_w_o, B_x, B_k_cache, B_v_cache, B_wq, B_wo,
):
    return _run(A_x, A_c_kv, A_w_q, A_w_uk, A_w_uv, A_w_o, B_x, B_k_cache, B_v_cache, B_wq, B_wo)
```

```python
import jax
import jax.numpy as jnp
import jax.experimental.pallas as pl
import jax.experimental.pallas.tpu as pltpu

B, H, SK, D, M, DC = 4, 32, 4096, 128, 512, 512
T = 128
NJ = SK // T
NT = (((1,), (1,)), ((), ()))
F32, BF16, U32 = jnp.float32, jnp.bfloat16, jnp.uint32
SIDE_BYTES = 4 * 1024 * 1024


def build(nbuf=4, HG=32, S=1, rows=64, prio="01", xkb=16, un=8, ntail=4, gmajor=False, nocomp=0, NQ=8, NQW=4):
    G = H // HG
    NS = NJ * G
    npc = (HG // S) * (T // rows)
    un = min(un, npc)
    xbytes = xkb * 1024
    NQ2 = 2 * NQ
    assert NQW * ntail <= H and SK // NQ >= 256

    def kernel(ax_h, ckv_h, awq_h, wuk_h, wuv_h, awo_h, bx_h, k_h, v_h, bwq_h, bwo_h,
               out_ref,
               ax_v, bx_v, ckv_v, awq_v, wuk_v, wuv_v, awo_v, bwq_v, bwo_v, ring,
               qb_s, s_s, p_s, oacc_s, ob_s, qabs_s, sa_s, pa_s, cacc_s, ctxc_s, ctx_s, outa_s,
               ring_sem, w_sem, x_sem, tail_sem):
        sub8 = jax.lax.broadcasted_iota(jnp.int32, (8, 128), 0)

        def loop(n, body):
            jax.lax.fori_loop(0, n, lambda i, c: (body(i), c)[1], 0)

        def split(i):
            return (i % NJ, i // NJ) if gmajor else (i // G, i % G)

        def issue_kv(src, i, slot):
            j, g = split(i)
            nh = HG // S

            def some(it):
                for u in range(un):
                    q = it * un + u
                    h, r = (q % nh) * S, (q // nh) * rows
                    r = pl.multiple_of(r, rows)
                    pltpu.make_async_copy(
                        src.at[pl.ds(g * HG + h, S), pl.ds(pl.multiple_of(j * T + r, rows), rows)],
                        ring.at[slot, pl.ds(h, S), pl.ds(r, rows)],
                        ring_sem.at[slot]).start(priority=int(prio[u % len(prio)]))
            loop(npc // un, some)

        def issue_part(src, dst, sem, i, n):
            nq, r, c = src.shape
            pr = 16
            pc = min(c, 512)
            seg = pr * pc * src.dtype.itemsize
            sq = xbytes // seg
            nc, ng = c // pc, nq // sq
            total = (r // pr) * nc * ng
            per = total // n
            u_n = min(un, per)

            def some(it):
                for u in range(u_n):
                    q = i * per + it * u_n + u
                    g, q = q % ng, q // ng
                    idx = (pl.ds(g * sq, sq), pl.ds(pl.multiple_of((q // nc) * pr, pr), pr),
                           pl.ds(pl.multiple_of((q % nc) * pc, pc), pc) if nc > 1 else slice(None))
                    pltpu.make_async_copy(src.at[idx], dst.at[idx], sem).start(
                        priority=int(prio[u % len(prio)]))
            loop(per // u_n, some)

        side = [[(awq_h.bitcast(U32), awq_v, 0), (wuk_h.bitcast(U32), wuk_v, 1)]]
        side += [[(ckv_h.at[b], ckv_v.at[b], 2 + b)] for b in range(B)]
        side += [[(wuv_h.bitcast(U32), wuv_v, 6)], [(awo_h, awo_v, 7)], []]

        def issue_side(p, i, parity=None):
            for pp in range(2 * B):
                if side[pp] and (parity is None or pp % 2 == parity):
                    @pl.when(p == pp)
                    def _(pp=pp):
                        for src, dst, s in side[pp]:
                            issue_part(src, dst, w_sem.at[s], i, NS)

        def wait_side(p, parity):
            for pp in range(2 * B):
                if side[pp] and pp % 2 == parity:
                    @pl.when(p == pp)
                    def _(pp=pp):
                        for src, dst, s in side[pp]:
                            pltpu.make_async_copy(dst, dst, w_sem.at[s]).wait()

        def issue_tail(t):
            per = -(-ntail // nbuf)

            def one(u):
                c = t * per + u

                @pl.when(c < ntail)
                def _():
                    issue_part(bwo_h, bwo_v, tail_sem.at[c], c, ntail)
            loop(per, one)

        def issue_ahead(b, v, i, slot):
            nxt = i + nbuf

            @pl.when(nxt < NS)
            def _():
                issue_kv((v_h if v else k_h).at[b], nxt, slot)
                issue_side(2 * b + v, nxt, v)

            @pl.when(nxt >= NS)
            def _():
                if v == 0:
                    issue_kv(v_h.at[b], nxt - NS, slot)
                    issue_side(2 * b + 1, nxt - NS, 1)
                else:
                    @pl.when(b + 1 < B)
                    def _():
                        issue_kv(k_h.at[b + 1], nxt - NS, slot)
                        issue_side(2 * b + 2, nxt - NS, 0)

                    @pl.when(b + 1 == B)
                    def _():
                        issue_tail(nxt - NS)

        cbx = pltpu.make_async_copy(bx_h, bx_v, x_sem.at[0])
        cax = pltpu.make_async_copy(ax_h, ax_v, x_sem.at[1])
        cbx.start()
        cax.start()
        issue_part(bwq_h, bwq_v, w_sem.at[8], 0, 1)

        def first(i):
            issue_kv(k_h.at[0], i, i)
            for src, dst, s in side[0]:
                issue_part(src, dst, w_sem.at[s], i, NS)
        loop(nbuf, first)

        ob_s[...] = jnp.zeros_like(ob_s)
        ctxc_s[...] = jnp.zeros_like(ctxc_s)
        outa_s[...] = jnp.zeros_like(outa_s)
        cbx.wait()
        cax.wait()
        pltpu.make_async_copy(bwq_v, bwq_v, w_sem.at[8]).wait()

        def pad8(x):
            return jnp.concatenate([x.astype(F32), jnp.zeros((8 - B, M), F32)], axis=0).astype(BF16)

        xb = pad8(bx_v[...])

        def qb_heads(i):
            w = bwq_v[:, :, pl.ds(pl.multiple_of(i * (4 * D), 4 * D), 4 * D)].reshape(M, 4 * D)
            r = jnp.dot(xb, w, preferred_element_type=F32)
            for e in range(4):
                qb_s[pl.ds(pl.multiple_of((i * 4 + e) * 8, 8), 8), :] = r[:, e * D:(e + 1) * D]
        loop(H // 4, qb_heads)

        def halves(ref, hp):
            u = jnp.concatenate(
                [ref[q, pl.ds(hp, M // NQ2, stride=H // 2), :] for q in range(NQ2)], axis=0)
            lo = pltpu.bitcast(u << 16, F32).astype(BF16)
            hi = pltpu.bitcast(u & jnp.uint32(0xFFFF0000), F32).astype(BF16)
            return lo, hi

        def side_qabs(hp):
            xa = pad8(ax_v[...])
            wq = halves(awq_v, hp)
            wk = halves(wuk_v, hp)
            for e in range(2):
                q = jnp.dot(xa, wq[e], preferred_element_type=F32).astype(BF16)
                r = jax.lax.dot_general(q, wk[e], NT, preferred_element_type=F32)
                row = pl.multiple_of((2 * hp + e) * 8, 8)
                for c in range(DC // 128):
                    qabs_s[c, pl.ds(row, 8), :] = r[:, c * 128:(c + 1) * 128]

        def softmax(s):
            m = jnp.max(jnp.max(s, axis=0), axis=1, keepdims=True)
            e = jnp.exp(s - m[None])
            l = jnp.sum(jnp.sum(e, axis=0), axis=1, keepdims=True)
            return e * (1.0 / l)[None]

        def rows_of(ref, i, n):
            per = ref.shape[1] // n
            return ref[i // per, pl.ds(pl.multiple_of((i % per) * n, n), n), :]

        def side_attn(b, j):
            @pl.when(j < NA)
            def _():
                q = jnp.concatenate(
                    [qabs_s[c, pl.ds(b, H, stride=8), :] for c in range(DC // 128)], axis=1).astype(BF16)
                c_blk = rows_of(ckv_v.at[b], j, AK)
                sa_s[j] = jax.lax.dot_general(q, c_blk, NT, preferred_element_type=F32) * (D ** -0.5)

            @pl.when(j == NA - 1)
            def _():
                pa_s[...] = softmax(sa_s[...]).astype(BF16)
                cacc_s[...] = jnp.zeros_like(cacc_s)

            @pl.when(j >= NA)
            def _():
                jj = j - NA
                c_blk = rows_of(ckv_v.at[b], jj, AK)
                cacc_s[...] += jnp.dot(pa_s[jj], c_blk, preferred_element_type=F32)

            @pl.when(j == NJ - 1)
            def _():
                for c in range(DC // 128):
                    ctxc_s[c, pl.ds(b, H, stride=8), :] = cacc_s[:, c * 128:(c + 1) * 128]

        def side_ctx(hp):
            wv = halves(wuv_v, hp)
            for e in range(2):
                row = pl.multiple_of((2 * hp + e) * 8, 8)
                lhs = jnp.concatenate(
                    [ctxc_s[c, pl.ds(row, 8), :] for c in range(DC // 128)], axis=1).astype(BF16)
                ctx_s[pl.ds(row, 8), :] = jnp.dot(lhs, wv[e], preferred_element_type=F32)

        def side_outa(h):
            lhs = ctx_s[pl.ds(pl.multiple_of(h * 8, 8), 8), :].astype(BF16)
            w = rows_of(awo_v, h, D)
            outa_s[...] += jnp.dot(lhs, w, preferred_element_type=F32)

        def side_compute(p, j):
            pl.when((p == 1) & (j % 2 == 0))(lambda: side_qabs(j // 2))
            pl.when((p >= 2) & (p < 2 + B))(lambda: side_attn(p - 2, j))
            pl.when((p == 2 + B) & (j % 2 == 0))(lambda: side_ctx(j // 2))
            pl.when(p == 3 + B)(lambda: side_outa(j))

        def tiles(v, b, i, slot):
            j, g = split(i)
            for gg in range(HG // 8):
                h0 = pl.multiple_of(g * HG + gg * 8, 8)
                if v == 0:
                    lhs = qb_s[pl.ds(h0 * 8 + b, 8, stride=8), :].astype(BF16)
                else:
                    lhs = p_s[j, pl.ds(h0, 8), :].astype(BF16)
                acc = None
                for hh in range(8):
                    t = ring[slot, gg * 8 + hh]
                    if v == 0:
                        r = jax.lax.dot_general(lhs, t, NT, preferred_element_type=F32)
                    else:
                        r = jnp.dot(lhs, t, preferred_element_type=F32)
                    acc = r if acc is None else jnp.where(sub8 == hh, r, acc)
                if v == 0:
                    s_s[j, pl.ds(h0, 8), :] = acc * (D ** -0.5)
                else:
                    oacc_s[pl.ds(h0, 8), :] += acc

        def phase(p):
            b, v = p // 2, p % 2
            for par in range(2):
                wait_side(p - 1, par)

            @pl.when(v == 1)
            def _():
                p_s[...] = softmax(s_s[...])
                oacc_s[...] = jnp.zeros_like(oacc_s)

            def step(i):
                slot = (p * NS + i) % nbuf
                pltpu.make_async_copy(ring.at[slot], ring.at[slot], ring_sem.at[slot]).wait()
                for vv in range(2):
                    @pl.when(v == vv)
                    def _(vv=vv):
                        if not nocomp & 1:
                            tiles(vv, b, i, slot)
                        issue_ahead(b, vv, i, slot)
                if nocomp & 2:
                    pass
                elif G == 1:
                    side_compute(p, i)
                else:
                    pl.when(i % G == 0)(lambda: side_compute(p, i // G))
            loop(NS, step)

            @pl.when(v == 1)
            def _():
                ob_s[pl.ds(b, H, stride=8), :] = oacc_s[...]

        loop(2 * B, phase)

        hq = H // NQW
        rc = hq * D // ntail

        def tail(c, acc):
            rows_c = pl.ds(pl.multiple_of(c * rc, rc), rc)
            pltpu.make_async_copy(bwo_v.at[:, rows_c], bwo_v.at[:, rows_c], tail_sem.at[c]).wait()
            k = rc // D
            for q in range(0 if nocomp & 4 else NQW):
                for e in range(k):
                    hh = c * k + e
                    lhs = ob_s[pl.ds(pl.multiple_of((q * hq + hh) * 8, 8), 8), :].astype(BF16)
                    acc += jnp.dot(lhs, bwo_v[q, pl.ds(pl.multiple_of(hh * D, D), D), :],
                                   preferred_element_type=F32)
            return acc
        outb = jax.lax.fori_loop(0, ntail, tail, jnp.zeros((8, M), F32))
        out_ref[:, 0:M] = outa_s[0:B, :].astype(out_ref.dtype)
        out_ref[:, M:2 * M] = outb[0:B, :].astype(out_ref.dtype)

    hbm = pl.BlockSpec(memory_space=pltpu.HBM)
    NA = NJ // 2
    AK = SK // NA

    def run(A_x, A_c_kv, A_w_q, A_w_uk, A_w_uv, A_w_o, B_x, B_k_cache, B_v_cache, B_wq, B_wo):
        out = pl.pallas_call(
            kernel,
            out_shape=jax.ShapeDtypeStruct((B, 2 * M), A_x.dtype),
            in_specs=[hbm] * 11,
            out_specs=pl.BlockSpec(memory_space=pltpu.VMEM),
            scratch_shapes=[
                pltpu.VMEM((B, M), BF16), pltpu.VMEM((B, M), BF16),
                pltpu.VMEM((B, NQ, SK // NQ, DC), BF16),
                pltpu.VMEM((NQ2, M * H // 2 // NQ2, D), U32), pltpu.VMEM((NQ2, DC * H // 2 // NQ2, D), U32),
                pltpu.VMEM((NQ2, DC * H // 2 // NQ2, D), U32),
                pltpu.VMEM((NQ, H * D // NQ, M), BF16), pltpu.VMEM((NQ, M // NQ, H * D), BF16),
                pltpu.VMEM((NQW, H * D // NQW, M), BF16),
                pltpu.VMEM((nbuf, HG, T, D), BF16),
                pltpu.VMEM((H * 8, D), F32),
                pltpu.VMEM((NJ, H, T), F32),
                pltpu.VMEM((NJ, H, T), F32),
                pltpu.VMEM((H, D), F32),
                pltpu.VMEM((H * 8, D), F32),
                pltpu.VMEM((DC // 128, H * 8, 128), F32),
                pltpu.VMEM((NA, H, AK), F32),
                pltpu.VMEM((NA, H, AK), BF16),
                pltpu.VMEM((H, DC), F32),
                pltpu.VMEM((DC // 128, H * 8, 128), F32),
                pltpu.VMEM((H * 8, D), F32),
                pltpu.VMEM((8, M), F32),
                pltpu.SemaphoreType.DMA((nbuf,)),
                pltpu.SemaphoreType.DMA((9,)),
                pltpu.SemaphoreType.DMA((2,)),
                pltpu.SemaphoreType.DMA((ntail,)),
            ],
            compiler_params=pltpu.CompilerParams(
                vmem_limit_bytes=100 * 1024 * 1024, disable_bounds_checks=True),
        )(A_x.reshape(B, M), A_c_kv.reshape(B, NQ, -1, DC), A_w_q.reshape(NQ2, -1, D),
          A_w_uk.reshape(NQ2, -1, D), A_w_uv.reshape(NQ2, -1, D), A_w_o.reshape(NQ, -1, M),
          B_x.reshape(B, M), B_k_cache, B_v_cache, B_wq.reshape(NQ, -1, H * D), B_wo.reshape(NQW, -1, M))
        return out.reshape(B, 1, 2 * M)

    return run


_run = build(HG=16, nbuf=8, S=4, rows=32, un=16, gmajor=True, xkb=16, NQ=16, NQW=8, ntail=4)


@jax.jit
def pallas_concat_heads__compressed_kv_cla__mha_block_cached__decode_kernel(
    A_x, A_c_kv, A_w_q, A_w_uk, A_w_uv, A_w_o, B_x, B_k_cache, B_v_cache, B_wq, B_wo,
):
    return _run(A_x, A_c_kv, A_w_q, A_w_uk, A_w_uv, A_w_o, B_x, B_k_cache, B_v_cache, B_wq, B_wo)
```

```python
import jax
import jax.numpy as jnp
import jax.experimental.pallas as pl
import jax.experimental.pallas.tpu as pltpu

B, H, SK, D, M, DC = 4, 32, 4096, 128, 512, 512
F32, BF16, U32 = jnp.float32, jnp.bfloat16, jnp.uint32
NT = (((1,), (1,)), ((), ()))
SCALE = D ** -0.5

T = 128
NJ = SK // T
HG = 16
G = H // HG
NS = NJ * G
NBUF = 8
PH, PR = 4, 32
NQ = 4
SIDE_PIECE = 32 * 1024
EDGE_PIECE = 16 * 1024
NTAIL = 8
NA = NJ // 2
AK = SK // NA


def _loop(n, body):
    def step(i, carry):
        body(i)
        return carry
    jax.lax.fori_loop(0, n, step, 0)


def _aligned(i, n):
    return pl.ds(pl.multiple_of(i * n, n), n)


def _rows_of(ref, i, n):
    per = ref.shape[1] // n
    return ref[i // per, _aligned(i % per, n), :]


def _pad_rows(x):
    return jnp.concatenate([x.astype(F32), jnp.zeros((8 - B, M), F32)], axis=0).astype(BF16)


def _softmax(s):
    m = jnp.max(jnp.max(s, axis=0), axis=1, keepdims=True)
    e = jnp.exp(s - m[None])
    l = jnp.sum(jnp.sum(e, axis=0), axis=1, keepdims=True)
    return e * (1.0 / l)[None]


def _wait_all(buf, sem):
    pltpu.make_async_copy(buf, buf, sem).wait()


def _start_parts(arrays, i, n, piece_bytes):
    nq, r, c = arrays[0][0].shape
    per = nq * r * c * 2 // piece_bytes // n
    unroll = min(16 // len(arrays), per)

    def some(it):
        k = 0
        for u in range(unroll):
            for src, dst, sem in arrays:
                c = src.shape[2]
                pc = min(c, 512)
                pr = max(16, 4096 // c)
                sq = piece_bytes // (pr * pc * 2)
                nc, ng = c // pc, nq // sq
                q = i * per + it * unroll + u
                g, q = q % ng, q // ng
                idx = (pl.ds(g * sq, sq), _aligned(q // nc, pr),
                       _aligned(q % nc, pc) if nc > 1 else slice(None))
                pltpu.make_async_copy(src.at[idx], dst.at[idx], sem).start(priority=k % 2)
                k += 1
    _loop(per // unroll, some)


def _kernel(ax_h, ckv_h, awq_h, wuk_h, wuv_h, awo_h, bx_h, k_h, v_h, bwq_h, bwo_h,
            out_ref,
            ax_v, bx_v, ckv_v, awq_v, wuk_v, wuv_v, awo_v, bwq_v, bwo_v, ring, pair0_s, pair1_s,
            qb_s, s_s, p_s, oacc_s, ob_s, qabs_s, sa_s, pa_s, cacc_s, ctxc_s, ctx_s, outa_s,
            ring_sem, w_sem, x_sem, tail_sem):
    sub8 = jax.lax.broadcasted_iota(jnp.int32, (8, 128), 0)

    side = [[(awq_h, awq_v, w_sem.at[0]), (wuk_h, wuk_v, w_sem.at[1])]]
    side += [[(ckv_h.at[b + e], ckv_v.at[b + e], w_sem.at[2 + b + e]) for e in range(2)]
             for b in range(0, B, 2)]
    side += [[(wuv_h, wuv_v, w_sem.at[6]), (awo_h, awo_v, w_sem.at[7])]]

    def start_kv(src, i, slot):
        j, g = i % NJ, i // NJ
        k = 0
        for r in range(0, T, PR):
            for h in range(0, HG, PH):
                pltpu.make_async_copy(
                    src.at[pl.ds(g * HG + h, PH), pl.ds(pl.multiple_of(j * T + r, PR), PR)],
                    ring.at[slot, pl.ds(h, PH), pl.ds(r, PR)],
                    ring_sem.at[slot]).start(priority=k % 2)
                k += 1

    def start_side(p, parity, i):
        for pp in range(parity, len(side), 2):
            pl.when(p == pp)(lambda pp=pp: _start_parts(side[pp], i, NS, SIDE_PIECE))

    def wait_side(p):
        for pp in range(len(side)):
            @pl.when(p == pp)
            def _(pp=pp):
                for _, dst, sem in side[pp]:
                    _wait_all(dst, sem)

    def start_ahead(b, v, i, slot):
        nxt = i + NBUF

        @pl.when(nxt < NS)
        def _():
            start_kv((v_h if v else k_h).at[b], nxt, slot)
            start_side(2 * b + v, v, nxt)

        @pl.when(nxt >= NS)
        def _():
            if v == 0:
                start_kv(v_h.at[b], nxt - NS, slot)
                start_side(2 * b + 1, 1, nxt - NS)
            else:
                @pl.when(b + 1 < B)
                def _():
                    start_kv(k_h.at[b + 1], nxt - NS, slot)
                    start_side(2 * b + 2, 0, nxt - NS)

                @pl.when((b + 1 == B) & (nxt - NS < NTAIL))
                def _():
                    _start_parts([(bwo_h, bwo_v, tail_sem.at[nxt - NS])], nxt - NS, NTAIL, EDGE_PIECE)

    copy_bx = pltpu.make_async_copy(bx_h, bx_v, x_sem.at[0])
    copy_ax = pltpu.make_async_copy(ax_h, ax_v, x_sem.at[1])
    copy_bx.start(priority=0)
    copy_ax.start(priority=1)
    _start_parts([(bwq_h, bwq_v, w_sem.at[8])], 0, 1, EDGE_PIECE)

    def first(i):
        start_kv(k_h.at[0], i, i)
        start_side(0 * i, 0, i)
    _loop(NBUF, first)

    ob_s[...] = jnp.zeros_like(ob_s)
    ctxc_s[...] = jnp.zeros_like(ctxc_s)
    outa_s[...] = jnp.zeros_like(outa_s)
    copy_bx.wait()
    copy_ax.wait()
    _wait_all(bwq_v, w_sem.at[8])

    xb = _pad_rows(bx_v[...])

    def mha_queries(i):
        w = bwq_v[:, :, _aligned(i, 4 * D)].reshape(M, 4 * D)
        r = jnp.dot(xb, w, preferred_element_type=F32)
        for e in range(4):
            qb_s[_aligned(i * 4 + e, 8), :] = r[:, e * D:(e + 1) * D]
    _loop(H // 4, mha_queries)

    def to_pairs(dst, src, i):
        n = M * H // (H // 2)
        dst[_aligned(i, n // 2), :] = pltpu.bitcast(_rows_of(src, i, n), U32)

    def head_pair(ref, hp):
        u = ref[pl.ds(hp, M, stride=H // 2), :]
        even = pltpu.bitcast(u << 16, F32).astype(BF16)
        odd = pltpu.bitcast(u & jnp.uint32(0xFFFF0000), F32).astype(BF16)
        return even, odd

    def latent_queries(hp):
        xa = _pad_rows(ax_v[...])
        wq = head_pair(pair0_s, hp)
        wk = head_pair(pair1_s, hp)
        for e in range(2):
            q = jnp.dot(xa, wq[e], preferred_element_type=F32).astype(BF16)
            r = jax.lax.dot_general(q, wk[e], NT, preferred_element_type=F32)
            for c in range(DC // 128):
                qabs_s[c, _aligned(2 * hp + e, 8), :] = r[:, c * 128:(c + 1) * 128]

    def latent_attention(b, j):
        @pl.when(j < NA)
        def _():
            q = jnp.concatenate(
                [qabs_s[c, pl.ds(b, H, stride=8), :] for c in range(DC // 128)], axis=1).astype(BF16)
            s = jax.lax.dot_general(q, _rows_of(ckv_v.at[b], j, AK), NT, preferred_element_type=F32)
            sa_s[j] = s * SCALE

        @pl.when(j == NA - 1)
        def _():
            pa_s[...] = _softmax(sa_s[...]).astype(BF16)
            cacc_s[...] = jnp.zeros_like(cacc_s)

        @pl.when(j >= NA)
        def _():
            cacc_s[...] += jnp.dot(pa_s[j - NA], _rows_of(ckv_v.at[b], j - NA, AK),
                                   preferred_element_type=F32)

        @pl.when(j == NJ - 1)
        def _():
            for c in range(DC // 128):
                ctxc_s[c, pl.ds(b, H, stride=8), :] = cacc_s[:, c * 128:(c + 1) * 128]

    def latent_context(hp):
        wv = head_pair(pair0_s, hp)
        for e in range(2):
            rows = _aligned(2 * hp + e, 8)
            lhs = jnp.concatenate([ctxc_s[c, rows, :] for c in range(DC // 128)], axis=1).astype(BF16)
            ctx_s[rows, :] = jnp.dot(lhs, wv[e], preferred_element_type=F32)

    def latent_output(h):
        outa_s[...] += jnp.dot(ctx_s[_aligned(h, 8), :].astype(BF16), _rows_of(awo_v, h, D),
                               preferred_element_type=F32)

    def latent_step(p, j):
        @pl.when((p == 1) & (j < H // 2))
        def _():
            to_pairs(pair0_s, awq_v, j)
            to_pairs(pair1_s, wuk_v, j)
        pl.when((p == 1) & (j >= H // 2))(lambda: latent_queries(j - H // 2))
        pl.when((p >= 2) & (p < 2 + B))(lambda: latent_attention(p - 2, j))
        pl.when((p == 2 + B) & (j < H // 2))(lambda: to_pairs(pair0_s, wuv_v, j))
        pl.when((p == 2 + B) & (j >= H // 2))(lambda: latent_context(j - H // 2))
        pl.when(p == 3 + B)(lambda: latent_output(j))

    def tiles(v, b, i, slot):
        j, g = i % NJ, i // NJ
        for gg in range(HG // 8):
            heads = g * (HG // 8) + gg
            if v == 0:
                lhs = qb_s[pl.ds(heads * 64 + b, 8, stride=8), :].astype(BF16)
            else:
                lhs = p_s[j, _aligned(heads, 8), :].astype(BF16)
            acc = None
            for hh in range(8):
                t = ring[slot, gg * 8 + hh]
                if v == 0:
                    r = jax.lax.dot_general(lhs, t, NT, preferred_element_type=F32)
                else:
                    r = jnp.dot(lhs, t, preferred_element_type=F32)
                acc = r if acc is None else jnp.where(sub8 == hh, r, acc)
            if v == 0:
                s_s[j, _aligned(heads, 8), :] = acc * SCALE
            else:
                oacc_s[_aligned(heads, 8), :] += acc

    def phase(p):
        b, v = p // 2, p % 2
        wait_side(p - 1)

        @pl.when(v == 1)
        def _():
            p_s[...] = _softmax(s_s[...])
            oacc_s[...] = jnp.zeros_like(oacc_s)

        def step(i):
            slot = i % NBUF
            _wait_all(ring.at[slot], ring_sem.at[slot])
            for vv in range(2):
                @pl.when(v == vv)
                def _(vv=vv):
                    tiles(vv, b, i, slot)
                    start_ahead(b, vv, i, slot)
            pl.when(i % G == 0)(lambda: latent_step(p, i // G))
        _loop(NS, step)

        @pl.when(v == 1)
        def _():
            ob_s[pl.ds(b, H, stride=8), :] = oacc_s[...]

    _loop(2 * B, phase)

    heads_per_part = H // NQ
    k = heads_per_part // NTAIL

    def tail(c, acc):
        _wait_all(bwo_v.at[:, _aligned(c, k * D)], tail_sem.at[c])
        for q in range(NQ):
            for e in range(k):
                hh = c * k + e
                lhs = ob_s[_aligned(q * heads_per_part + hh, 8), :].astype(BF16)
                acc += jnp.dot(lhs, bwo_v[q, _aligned(hh, D), :], preferred_element_type=F32)
        return acc
    out_b = jax.lax.fori_loop(0, NTAIL, tail, jnp.zeros((8, M), F32))
    out_ref[:, 0:M] = outa_s[0:B, :].astype(out_ref.dtype)
    out_ref[:, M:2 * M] = out_b[0:B, :].astype(out_ref.dtype)


assert NS % NBUF == 0 and NTAIL <= NBUF and H % (NQ * NTAIL) == 0 and NJ == H


@jax.jit
def pallas_concat_heads__compressed_kv_cla__mha_block_cached__decode_kernel(
    A_x: jax.Array,
    A_c_kv: jax.Array,
    A_w_q: jax.Array,
    A_w_uk: jax.Array,
    A_w_uv: jax.Array,
    A_w_o: jax.Array,
    B_x: jax.Array,
    B_k_cache: jax.Array,
    B_v_cache: jax.Array,
    B_wq: jax.Array,
    B_wo: jax.Array,
):
    out = pl.pallas_call(
        _kernel,
        out_shape=jax.ShapeDtypeStruct((B, 2 * M), A_x.dtype),
        in_specs=[pl.BlockSpec(memory_space=pltpu.HBM)] * 11,
        out_specs=pl.BlockSpec(memory_space=pltpu.VMEM),
        scratch_shapes=[
            pltpu.VMEM((B, M), BF16),
            pltpu.VMEM((B, M), BF16),
            pltpu.VMEM((B, NQ, SK // NQ, DC), BF16),
            pltpu.VMEM((NQ, M * H // NQ, D), BF16),
            pltpu.VMEM((NQ, DC * H // NQ, D), BF16),
            pltpu.VMEM((NQ, DC * H // NQ, D), BF16),
            pltpu.VMEM((NQ, H * D // NQ, M), BF16),
            pltpu.VMEM((NQ, M // NQ, H * D), BF16),
            pltpu.VMEM((NQ, H * D // NQ, M), BF16),
            pltpu.VMEM((NBUF, HG, T, D), BF16),
            pltpu.VMEM((M * H // 2, D), U32),
            pltpu.VMEM((DC * H // 2, D), U32),
            pltpu.VMEM((H * 8, D), F32),
            pltpu.VMEM((NJ, H, T), F32),
            pltpu.VMEM((NJ, H, T), F32),
            pltpu.VMEM((H, D), F32),
            pltpu.VMEM((H * 8, D), F32),
            pltpu.VMEM((DC // 128, H * 8, 128), F32),
            pltpu.VMEM((NA, H, AK), F32),
            pltpu.VMEM((NA, H, AK), BF16),
            pltpu.VMEM((H, DC), F32),
            pltpu.VMEM((DC // 128, H * 8, 128), F32),
            pltpu.VMEM((H * 8, D), F32),
            pltpu.VMEM((8, M), F32),
            pltpu.SemaphoreType.DMA((NBUF,)),
            pltpu.SemaphoreType.DMA((9,)),
            pltpu.SemaphoreType.DMA((2,)),
            pltpu.SemaphoreType.DMA((NTAIL,)),
        ],
        compiler_params=pltpu.CompilerParams(
            vmem_limit_bytes=80 * 1024 * 1024, disable_bounds_checks=True),
    )(A_x.reshape(B, M), A_c_kv.reshape(B, NQ, -1, DC), A_w_q.reshape(NQ, -1, D),
      A_w_uk.reshape(NQ, -1, D), A_w_uv.reshape(NQ, -1, D), A_w_o.reshape(NQ, -1, M),
      B_x.reshape(B, M), B_k_cache, B_v_cache, B_wq.reshape(NQ, -1, H * D), B_wo.reshape(NQ, -1, M))
    return out.reshape(B, 1, 2 * M)
```

```python
import jax
import jax.numpy as jnp
import jax.experimental.pallas as pl
import jax.experimental.pallas.tpu as pltpu

B, H, SK, D, M, DC = 4, 32, 4096, 128, 512, 512
F32, BF16, U32 = jnp.float32, jnp.bfloat16, jnp.uint32
NT = (((1,), (1,)), ((), ()))
SCALE = D ** -0.5

T = 128
NJ = SK // T
HG = 16
G = H // HG
NS = NJ * G
NBUF = 8
PH, PR = 4, 32
NQ = 4
SIDE_PIECE = 32 * 1024
EDGE_PIECE = 16 * 1024
NTAIL = 8
NA = NJ // 2
AK = SK // NA


def _loop(n, body):
    def step(i, carry):
        body(i)
        return carry
    jax.lax.fori_loop(0, n, step, 0)


def _aligned(i, n):
    return pl.ds(pl.multiple_of(i * n, n), n)


def _rows_of(ref, i, n):
    per = ref.shape[1] // n
    return ref[i // per, _aligned(i % per, n), :]


def _pad_rows(x):
    return jnp.concatenate([x.astype(F32), jnp.zeros((8 - B, M), F32)], axis=0).astype(BF16)


def _softmax(s):
    m = jnp.max(jnp.max(s, axis=0), axis=1, keepdims=True)
    e = jnp.exp(s - m[None])
    l = jnp.sum(jnp.sum(e, axis=0), axis=1, keepdims=True)
    return e * (1.0 / l)[None]


def _wait_all(buf, sem):
    pltpu.make_async_copy(buf, buf, sem).wait()


def _start_parts(arrays, i, n, piece_bytes):
    nq, r, c = arrays[0][0].shape
    per = nq * r * c * 2 // piece_bytes // n
    unroll = min(16 // len(arrays), per)

    def some(it):
        k = 0
        for u in range(unroll):
            for src, dst, sem in arrays:
                c = src.shape[2]
                pc = min(c, 512)
                pr = max(16, 4096 // c)
                sq = piece_bytes // (pr * pc * 2)
                nc, ng = c // pc, nq // sq
                q = i * per + it * unroll + u
                g, q = q % ng, q // ng
                idx = (pl.ds(g * sq, sq), _aligned(q // nc, pr),
                       _aligned(q % nc, pc) if nc > 1 else slice(None))
                pltpu.make_async_copy(src.at[idx], dst.at[idx], sem).start(priority=k % 2)
                k += 1
    _loop(per // unroll, some)


def _kernel(ax_h, ckv_h, awq_h, wuk_h, wuv_h, awo_h, bx_h, k_h, v_h, bwq_h, bwo_h,
            out_ref,
            ax_v, bx_v, ckv_v, awq_v, wuk_v, wuv_v, awo_v, bwq_v, bwo_v, ring, pair0_s, pair1_s,
            qb_s, s_s, p_s, oacc_s, ob_s, qabs_s, sa_s, pa_s, cacc_s, ctxc_s, ctx_s, outa_s,
            ring_sem, w_sem, x_sem, tail_sem):
    sub8 = jax.lax.broadcasted_iota(jnp.int32, (8, 128), 0)

    side = [[(awq_h, awq_v, w_sem.at[0]), (wuk_h, wuk_v, w_sem.at[1])]]
    side += [[(ckv_h.at[b + e], ckv_v.at[b + e], w_sem.at[2 + b + e]) for e in range(2)]
             for b in range(0, B, 2)]
    side += [[(wuv_h, wuv_v, w_sem.at[6]), (awo_h, awo_v, w_sem.at[7])]]

    def start_kv(src, i, slot):
        j, g = i % NJ, i // NJ
        k = 0
        for r in range(0, T, PR):
            for h in range(0, HG, PH):
                pltpu.make_async_copy(
                    src.at[pl.ds(g * HG + h, PH), pl.ds(pl.multiple_of(j * T + r, PR), PR)],
                    ring.at[slot, pl.ds(h, PH), pl.ds(r, PR)],
                    ring_sem.at[slot]).start(priority=k % 2)
                k += 1

    def start_side(p, parity, i):
        for pp in range(parity, len(side), 2):
            pl.when(p == pp)(lambda pp=pp: _start_parts(side[pp], i, NS, SIDE_PIECE))

    def wait_side(p):
        for pp in range(len(side)):
            @pl.when(p == pp)
            def _(pp=pp):
                for _, dst, sem in side[pp]:
                    _wait_all(dst, sem)

    def start_ahead(b, v, i, slot):
        nxt = i + NBUF

        @pl.when(nxt < NS)
        def _():
            start_kv((v_h if v else k_h).at[b], nxt, slot)
            start_side(2 * b + v, v, nxt)

        @pl.when(nxt >= NS)
        def _():
            if v == 0:
                start_kv(v_h.at[b], nxt - NS, slot)
                start_side(2 * b + 1, 1, nxt - NS)
            else:
                @pl.when(b + 1 < B)
                def _():
                    start_kv(k_h.at[b + 1], nxt - NS, slot)
                    start_side(2 * b + 2, 0, nxt - NS)

                @pl.when((b + 1 == B) & (nxt - NS < NTAIL))
                def _():
                    _start_parts([(bwo_h, bwo_v, tail_sem.at[nxt - NS])], nxt - NS, NTAIL, EDGE_PIECE)

    copy_bx = pltpu.make_async_copy(bx_h, bx_v, x_sem.at[0])
    copy_ax = pltpu.make_async_copy(ax_h, ax_v, x_sem.at[1])
    copy_bx.start(priority=0)
    copy_ax.start(priority=1)
    _start_parts([(bwq_h, bwq_v, w_sem.at[8])], 0, 1, EDGE_PIECE)

    def first(i):
        start_kv(k_h.at[0], i, i)
        _start_parts(side[0], i, NS, SIDE_PIECE)
    _loop(NBUF, first)

    ob_s[...] = jnp.zeros_like(ob_s)
    ctxc_s[...] = jnp.zeros_like(ctxc_s)
    outa_s[...] = jnp.zeros_like(outa_s)
    copy_bx.wait()
    copy_ax.wait()
    _wait_all(bwq_v, w_sem.at[8])

    xb = _pad_rows(bx_v[...])

    def mha_queries(i):
        w = bwq_v[:, :, _aligned(i, 4 * D)].reshape(M, 4 * D)
        r = jnp.dot(xb, w, preferred_element_type=F32)
        for e in range(4):
            qb_s[_aligned(i * 4 + e, 8), :] = r[:, e * D:(e + 1) * D]
    _loop(H // 4, mha_queries)

    def to_pairs(dst, src, i):
        n = M * H // (H // 2)
        dst[_aligned(i, n // 2), :] = pltpu.bitcast(_rows_of(src, i, n), U32)

    def head_pair(ref, hp):
        u = ref[pl.ds(hp, M, stride=H // 2), :]
        even = pltpu.bitcast(u << 16, F32).astype(BF16)
        odd = pltpu.bitcast(u & jnp.uint32(0xFFFF0000), F32).astype(BF16)
        return even, odd

    def latent_queries(hp):
        xa = _pad_rows(ax_v[...])
        wq = head_pair(pair0_s, hp)
        wk = head_pair(pair1_s, hp)
        for e in range(2):
            q = jnp.dot(xa, wq[e], preferred_element_type=F32).astype(BF16)
            r = jax.lax.dot_general(q, wk[e], NT, preferred_element_type=F32)
            for c in range(DC // 128):
                qabs_s[c, _aligned(2 * hp + e, 8), :] = r[:, c * 128:(c + 1) * 128]

    def latent_attention(b, j):
        @pl.when(j < NA)
        def _():
            q = jnp.concatenate(
                [qabs_s[c, pl.ds(b, H, stride=8), :] for c in range(DC // 128)], axis=1).astype(BF16)
            s = jax.lax.dot_general(q, _rows_of(ckv_v.at[b], j, AK), NT, preferred_element_type=F32)
            sa_s[j] = s * SCALE

        @pl.when(j == NA - 1)
        def _():
            pa_s[...] = _softmax(sa_s[...]).astype(BF16)
            cacc_s[...] = jnp.zeros_like(cacc_s)

        @pl.when(j >= NA)
        def _():
            cacc_s[...] += jnp.dot(pa_s[j - NA], _rows_of(ckv_v.at[b], j - NA, AK),
                                   preferred_element_type=F32)

        @pl.when(j == NJ - 1)
        def _():
            for c in range(DC // 128):
                ctxc_s[c, pl.ds(b, H, stride=8), :] = cacc_s[:, c * 128:(c + 1) * 128]

    def latent_context(hp):
        wv = head_pair(pair0_s, hp)
        for e in range(2):
            rows = _aligned(2 * hp + e, 8)
            lhs = jnp.concatenate([ctxc_s[c, rows, :] for c in range(DC // 128)], axis=1).astype(BF16)
            ctx_s[rows, :] = jnp.dot(lhs, wv[e], preferred_element_type=F32)

    def latent_output(h):
        outa_s[...] += jnp.dot(ctx_s[_aligned(h, 8), :].astype(BF16), _rows_of(awo_v, h, D),
                               preferred_element_type=F32)

    def latent_step(p, j):
        @pl.when((p == 1) & (j < H // 2))
        def _():
            to_pairs(pair0_s, awq_v, j)
            to_pairs(pair1_s, wuk_v, j)
        pl.when((p == 1) & (j >= H // 2))(lambda: latent_queries(j - H // 2))
        pl.when((p >= 2) & (p < 2 + B))(lambda: latent_attention(p - 2, j))
        pl.when((p == 2 + B) & (j < H // 2))(lambda: to_pairs(pair0_s, wuv_v, j))
        pl.when((p == 2 + B) & (j >= H // 2))(lambda: latent_context(j - H // 2))
        pl.when(p == 3 + B)(lambda: latent_output(j))

    def tiles(v, b, i, slot):
        j, g = i % NJ, i // NJ
        for gg in range(HG // 8):
            heads = g * (HG // 8) + gg
            if v == 0:
                lhs = qb_s[pl.ds(heads * 64 + b, 8, stride=8), :].astype(BF16)
            else:
                lhs = p_s[j, _aligned(heads, 8), :].astype(BF16)
            acc = None
            for hh in range(8):
                t = ring[slot, gg * 8 + hh]
                if v == 0:
                    r = jax.lax.dot_general(lhs, t, NT, preferred_element_type=F32)
                else:
                    r = jnp.dot(lhs, t, preferred_element_type=F32)
                acc = r if acc is None else jnp.where(sub8 == hh, r, acc)
            if v == 0:
                s_s[j, _aligned(heads, 8), :] = acc * SCALE
            else:
                oacc_s[_aligned(heads, 8), :] += acc

    def phase(p):
        b, v = p // 2, p % 2
        wait_side(p - 1)

        @pl.when(v == 1)
        def _():
            p_s[...] = _softmax(s_s[...])
            oacc_s[...] = jnp.zeros_like(oacc_s)

        def step(i):
            slot = i % NBUF
            _wait_all(ring.at[slot], ring_sem.at[slot])
            for vv in range(2):
                @pl.when(v == vv)
                def _(vv=vv):
                    tiles(vv, b, i, slot)
                    start_ahead(b, vv, i, slot)
            pl.when(i % G == 0)(lambda: latent_step(p, i // G))
        _loop(NS, step)

        @pl.when(v == 1)
        def _():
            ob_s[pl.ds(b, H, stride=8), :] = oacc_s[...]

    _loop(2 * B, phase)

    heads_per_part = H // NQ
    k = heads_per_part // NTAIL

    def tail(c, acc):
        _wait_all(bwo_v.at[:, _aligned(c, k * D)], tail_sem.at[c])
        for q in range(NQ):
            for e in range(k):
                hh = c * k + e
                lhs = ob_s[_aligned(q * heads_per_part + hh, 8), :].astype(BF16)
                acc += jnp.dot(lhs, bwo_v[q, _aligned(hh, D), :], preferred_element_type=F32)
        return acc
    out_b = jax.lax.fori_loop(0, NTAIL, tail, jnp.zeros((8, M), F32))
    out_ref[:, 0:M] = outa_s[0:B, :].astype(out_ref.dtype)
    out_ref[:, M:2 * M] = out_b[0:B, :].astype(out_ref.dtype)


assert NS % NBUF == 0 and NTAIL <= NBUF and H % (NQ * NTAIL) == 0 and NJ == H


@jax.jit
def pallas_concat_heads__compressed_kv_cla__mha_block_cached__decode_kernel(
    A_x: jax.Array,
    A_c_kv: jax.Array,
    A_w_q: jax.Array,
    A_w_uk: jax.Array,
    A_w_uv: jax.Array,
    A_w_o: jax.Array,
    B_x: jax.Array,
    B_k_cache: jax.Array,
    B_v_cache: jax.Array,
    B_wq: jax.Array,
    B_wo: jax.Array,
):
    out = pl.pallas_call(
        _kernel,
        out_shape=jax.ShapeDtypeStruct((B, 2 * M), A_x.dtype),
        in_specs=[pl.BlockSpec(memory_space=pltpu.HBM)] * 11,
        out_specs=pl.BlockSpec(memory_space=pltpu.VMEM),
        scratch_shapes=[
            pltpu.VMEM((B, M), BF16),
            pltpu.VMEM((B, M), BF16),
            pltpu.VMEM((B, NQ, SK // NQ, DC), BF16),
            pltpu.VMEM((NQ, M * H // NQ, D), BF16),
            pltpu.VMEM((NQ, DC * H // NQ, D), BF16),
            pltpu.VMEM((NQ, DC * H // NQ, D), BF16),
            pltpu.VMEM((NQ, H * D // NQ, M), BF16),
            pltpu.VMEM((NQ, M // NQ, H * D), BF16),
            pltpu.VMEM((NQ, H * D // NQ, M), BF16),
            pltpu.VMEM((NBUF, HG, T, D), BF16),
            pltpu.VMEM(((M + 1) * H // 2, D), U32),
            pltpu.VMEM(((DC + 1) * H // 2, D), U32),
            pltpu.VMEM((H * 8 + 8, D), F32),
            pltpu.VMEM((NJ, H, T), F32),
            pltpu.VMEM((NJ, H, T), F32),
            pltpu.VMEM((H, D), F32),
            pltpu.VMEM((H * 8 + 8, D), F32),
            pltpu.VMEM((DC // 128, H * 8 + 8, 128), F32),
            pltpu.VMEM((NA, H, AK), F32),
            pltpu.VMEM((NA, H, AK), BF16),
            pltpu.VMEM((H, DC), F32),
            pltpu.VMEM((DC // 128, H * 8 + 8, 128), F32),
            pltpu.VMEM((H * 8, D), F32),
            pltpu.VMEM((8, M), F32),
            pltpu.SemaphoreType.DMA((NBUF,)),
            pltpu.SemaphoreType.DMA((9,)),
            pltpu.SemaphoreType.DMA((2,)),
            pltpu.SemaphoreType.DMA((NTAIL,)),
        ],
        compiler_params=pltpu.CompilerParams(
            vmem_limit_bytes=80 * 1024 * 1024, disable_bounds_checks=True),
    )(A_x.reshape(B, M), A_c_kv.reshape(B, NQ, -1, DC), A_w_q.reshape(NQ, -1, D),
      A_w_uk.reshape(NQ, -1, D), A_w_uv.reshape(NQ, -1, D), A_w_o.reshape(NQ, -1, M),
      B_x.reshape(B, M), B_k_cache, B_v_cache, B_wq.reshape(NQ, -1, H * D), B_wo.reshape(NQ, -1, M))
    return out.reshape(B, 1, 2 * M)
```

```python
import jax
import jax.numpy as jnp
import jax.experimental.pallas as pl
import jax.experimental.pallas.tpu as pltpu

B, H, SK, D, M, DC = 4, 32, 4096, 128, 512, 512
F32, BF16, U32 = jnp.float32, jnp.bfloat16, jnp.uint32
NT = (((1,), (1,)), ((), ()))
SCALE = D ** -0.5

T = 128
NJ = SK // T
NBUF = 4
PH, PR = 4, 32
NQ = 4
SIDE_PIECE = 32 * 1024
EDGE_PIECE = 16 * 1024
NTAIL = 8
NA = NJ // 2
AK = SK // NA


def _loop(n, body):
    def step(i, carry):
        body(i)
        return carry
    jax.lax.fori_loop(0, n, step, 0)


def _aligned(i, n):
    return pl.ds(pl.multiple_of(i * n, n), n)


def _rows_of(ref, i, n):
    per = ref.shape[1] // n
    return ref[i // per, _aligned(i % per, n), :]


def _pad_rows(x):
    return jnp.concatenate([x.astype(F32), jnp.zeros((8 - B, M), F32)], axis=0).astype(BF16)


def _softmax(s):
    m = jnp.max(jnp.max(s, axis=0), axis=1, keepdims=True)
    e = jnp.exp(s - m[None])
    l = jnp.sum(jnp.sum(e, axis=0), axis=1, keepdims=True)
    return e * (1.0 / l)[None]


def _wait_all(buf, sem):
    pltpu.make_async_copy(buf, buf, sem).wait()


def _start_parts(arrays, i, n, piece_bytes):
    nq, r, c = arrays[0][0].shape
    per = nq * r * c * 2 // piece_bytes // n
    unroll = min(16 // len(arrays), per)

    def some(it):
        k = 0
        for u in range(unroll):
            for src, dst, sem in arrays:
                c = src.shape[2]
                pc = min(c, 512)
                pr = max(16, 4096 // c)
                sq = piece_bytes // (pr * pc * 2)
                nc, ng = c // pc, nq // sq
                q = i * per + it * unroll + u
                g, q = q % ng, q // ng
                idx = (pl.ds(g * sq, sq), _aligned(q // nc, pr),
                       _aligned(q % nc, pc) if nc > 1 else slice(None))
                pltpu.make_async_copy(src.at[idx], dst.at[idx], sem).start(priority=k % 2)
                k += 1
    _loop(per // unroll, some)


def _kernel(ax_h, ckv_h, awq_h, wuk_h, wuv_h, awo_h, bx_h, k_h, v_h, bwq_h, bwo_h,
            out_ref,
            ax_v, bx_v, ckv_v, awq_v, wuk_v, wuv_v, awo_v, bwq_v, bwo_v, ring, pair0_s, pair1_s,
            qb_s, s_s, p_s, oacc_s, ob_s, qabs_s, sa_s, pa_s, cacc_s, ctxc_s, ctx_s, outa_s,
            ring_sem, w_sem, x_sem, tail_sem):
    sub8 = jax.lax.broadcasted_iota(jnp.int32, (8, 128), 0)

    side = [[(awq_h, awq_v, w_sem.at[0]), (wuk_h, wuk_v, w_sem.at[1])]]
    side += [[(ckv_h.at[b + e], ckv_v.at[b + e], w_sem.at[2 + b + e]) for e in range(2)]
             for b in range(0, B, 2)]
    side += [[(wuv_h, wuv_v, w_sem.at[6]), (awo_h, awo_v, w_sem.at[7])]]

    def start_kv(src, j, slot):
        k = 0
        for r in range(0, T, PR):
            for h in range(0, H, PH):
                pltpu.make_async_copy(
                    src.at[pl.ds(h, PH), pl.ds(pl.multiple_of(j * T + r, PR), PR)],
                    ring.at[slot, pl.ds(h, PH), pl.ds(r, PR)],
                    ring_sem.at[slot]).start(priority=k % 2)
                k += 1

    def start_side(p, parity, j):
        for pp in range(parity, len(side), 2):
            pl.when(p == pp)(lambda pp=pp: _start_parts(side[pp], j, NJ, SIDE_PIECE))

    def wait_side(p):
        for pp in range(len(side)):
            @pl.when(p == pp)
            def _(pp=pp):
                for _src, dst, sem in side[pp]:
                    _wait_all(dst, sem)

    def start_tail(c):
        _start_parts([(bwo_h, bwo_v, tail_sem.at[c])], c, NTAIL, EDGE_PIECE)

    def start_ahead(b, v, j, slot):
        nxt = j + NBUF

        @pl.when(nxt < NJ)
        def _():
            start_kv((v_h if v else k_h).at[b], nxt, slot)
            start_side(2 * b + v, v, nxt)

        @pl.when(nxt >= NJ)
        def _():
            if v == 0:
                start_kv(v_h.at[b], nxt - NJ, slot)
                start_side(2 * b + 1, 1, nxt - NJ)
            else:
                @pl.when(b + 1 < B)
                def _():
                    start_kv(k_h.at[b + 1], nxt - NJ, slot)
                    start_side(2 * b + 2, 0, nxt - NJ)

                @pl.when(b + 1 == B)
                def _():
                    per = NTAIL // NBUF
                    _loop(per, lambda u: start_tail((nxt - NJ) * per + u))

    copy_bx = pltpu.make_async_copy(bx_h, bx_v, x_sem.at[0])
    copy_ax = pltpu.make_async_copy(ax_h, ax_v, x_sem.at[1])
    copy_bx.start(priority=0)
    copy_ax.start(priority=1)
    _start_parts([(bwq_h, bwq_v, w_sem.at[8])], 0, 1, EDGE_PIECE)

    def first(j):
        start_kv(k_h.at[0], j, j)
        _start_parts(side[0], j, NJ, SIDE_PIECE)
    _loop(NBUF, first)

    ob_s[...] = jnp.zeros_like(ob_s)
    ctxc_s[...] = jnp.zeros_like(ctxc_s)
    outa_s[...] = jnp.zeros_like(outa_s)
    copy_bx.wait()
    copy_ax.wait()
    _wait_all(bwq_v, w_sem.at[8])

    xb = _pad_rows(bx_v[...])

    def mha_queries(i):
        w = bwq_v[:, :, _aligned(i, 4 * D)].reshape(M, 4 * D)
        r = jnp.dot(xb, w, preferred_element_type=F32)
        for e in range(4):
            qb_s[_aligned(i * 4 + e, 8), :] = r[:, e * D:(e + 1) * D]
    _loop(H // 4, mha_queries)

    def to_pairs(dst, src, i):
        n = M * H // (H // 2)
        dst[_aligned(i, n // 2), :] = pltpu.bitcast(_rows_of(src, i, n), U32)

    def head_pair(ref, hp):
        u = ref[pl.ds(hp, M, stride=H // 2), :]
        even = pltpu.bitcast(u << 16, F32).astype(BF16)
        odd = pltpu.bitcast(u & jnp.uint32(0xFFFF0000), F32).astype(BF16)
        return even, odd

    def latent_queries(hp):
        xa = _pad_rows(ax_v[...])
        wq = head_pair(pair0_s, hp)
        wk = head_pair(pair1_s, hp)
        for e in range(2):
            q = jnp.dot(xa, wq[e], preferred_element_type=F32).astype(BF16)
            r = jax.lax.dot_general(q, wk[e], NT, preferred_element_type=F32)
            for c in range(DC // 128):
                qabs_s[c, _aligned(2 * hp + e, 8), :] = r[:, c * 128:(c + 1) * 128]

    def latent_attention(b, j):
        @pl.when(j < NA)
        def _():
            q = jnp.concatenate(
                [qabs_s[c, pl.ds(b, H, stride=8), :] for c in range(DC // 128)], axis=1).astype(BF16)
            s = jax.lax.dot_general(q, _rows_of(ckv_v.at[b], j, AK), NT, preferred_element_type=F32)
            sa_s[j] = s * SCALE

        @pl.when(j == NA - 1)
        def _():
            pa_s[...] = _softmax(sa_s[...]).astype(BF16)
            cacc_s[...] = jnp.zeros_like(cacc_s)

        @pl.when(j >= NA)
        def _():
            cacc_s[...] += jnp.dot(pa_s[j - NA], _rows_of(ckv_v.at[b], j - NA, AK),
                                   preferred_element_type=F32)

        @pl.when(j == NJ - 1)
        def _():
            for c in range(DC // 128):
                ctxc_s[c, pl.ds(b, H, stride=8), :] = cacc_s[:, c * 128:(c + 1) * 128]

    def latent_context(hp):
        wv = head_pair(pair0_s, hp)
        for e in range(2):
            rows = _aligned(2 * hp + e, 8)
            lhs = jnp.concatenate([ctxc_s[c, rows, :] for c in range(DC // 128)], axis=1).astype(BF16)
            ctx_s[rows, :] = jnp.dot(lhs, wv[e], preferred_element_type=F32)

    def latent_output(h):
        outa_s[...] += jnp.dot(ctx_s[_aligned(h, 8), :].astype(BF16), _rows_of(awo_v, h, D),
                               preferred_element_type=F32)

    def latent_step(p, j):
        @pl.when((p == 1) & (j < H // 2))
        def _():
            to_pairs(pair0_s, awq_v, j)
            to_pairs(pair1_s, wuk_v, j)
        pl.when((p == 1) & (j >= H // 2))(lambda: latent_queries(j - H // 2))
        pl.when((p >= 2) & (p < 2 + B))(lambda: latent_attention(p - 2, j))
        pl.when((p == 2 + B) & (j < H // 2))(lambda: to_pairs(pair0_s, wuv_v, j))
        pl.when((p == 2 + B) & (j >= H // 2))(lambda: latent_context(j - H // 2))
        pl.when(p == 3 + B)(lambda: latent_output(j))

    def tiles(v, b, j, slot):
        for g in range(H // 8):
            heads = slice(g * 8, (g + 1) * 8)
            if v == 0:
                lhs = qb_s[pl.ds(g * 64 + b, 8, stride=8), :].astype(BF16)
            else:
                lhs = p_s[j, heads, :].astype(BF16)
            acc = None
            for hh in range(8):
                t = ring[slot, g * 8 + hh]
                if v == 0:
                    r = jax.lax.dot_general(lhs, t, NT, preferred_element_type=F32)
                else:
                    r = jnp.dot(lhs, t, preferred_element_type=F32)
                acc = r if acc is None else jnp.where(sub8 == hh, r, acc)
            if v == 0:
                s_s[j, heads, :] = acc * SCALE
            else:
                oacc_s[heads, :] += acc

    def phase(p):
        b, v = p // 2, p % 2
        wait_side(p - 1)

        @pl.when(v == 1)
        def _():
            p_s[...] = _softmax(s_s[...])
            oacc_s[...] = jnp.zeros_like(oacc_s)

        def step(j):
            slot = j % NBUF
            _wait_all(ring.at[slot], ring_sem.at[slot])
            for vv in range(2):
                @pl.when(v == vv)
                def _(vv=vv):
                    tiles(vv, b, j, slot)
                    start_ahead(b, vv, j, slot)
            latent_step(p, j)
        _loop(NJ, step)

        @pl.when(v == 1)
        def _():
            ob_s[pl.ds(b, H, stride=8), :] = oacc_s[...]

    _loop(2 * B, phase)

    heads_per_part = H // NQ
    k = heads_per_part // NTAIL

    def tail(c, acc):
        _wait_all(bwo_v.at[:, _aligned(c, k * D)], tail_sem.at[c])
        for q in range(NQ):
            for e in range(k):
                hh = c * k + e
                lhs = ob_s[_aligned(q * heads_per_part + hh, 8), :].astype(BF16)
                acc += jnp.dot(lhs, bwo_v[q, _aligned(hh, D), :], preferred_element_type=F32)
        return acc
    out_b = jax.lax.fori_loop(0, NTAIL, tail, jnp.zeros((8, M), F32))
    out_ref[:, 0:M] = outa_s[0:B, :].astype(out_ref.dtype)
    out_ref[:, M:2 * M] = out_b[0:B, :].astype(out_ref.dtype)


assert NJ % NBUF == 0 and NTAIL % NBUF == 0 and H % (NQ * NTAIL) == 0 and NJ == H


@jax.jit
def pallas_concat_heads__compressed_kv_cla__mha_block_cached__decode_kernel(
    A_x: jax.Array,
    A_c_kv: jax.Array,
    A_w_q: jax.Array,
    A_w_uk: jax.Array,
    A_w_uv: jax.Array,
    A_w_o: jax.Array,
    B_x: jax.Array,
    B_k_cache: jax.Array,
    B_v_cache: jax.Array,
    B_wq: jax.Array,
    B_wo: jax.Array,
):
    out = pl.pallas_call(
        _kernel,
        out_shape=jax.ShapeDtypeStruct((B, 2 * M), A_x.dtype),
        in_specs=[pl.BlockSpec(memory_space=pltpu.HBM)] * 11,
        out_specs=pl.BlockSpec(memory_space=pltpu.VMEM),
        scratch_shapes=[
            pltpu.VMEM((B, M), BF16),
            pltpu.VMEM((B, M), BF16),
            pltpu.VMEM((B, NQ, SK // NQ, DC), BF16),
            pltpu.VMEM((NQ, M * H // NQ, D), BF16),
            pltpu.VMEM((NQ, DC * H // NQ, D), BF16),
            pltpu.VMEM((NQ, DC * H // NQ, D), BF16),
            pltpu.VMEM((NQ, H * D // NQ, M), BF16),
            pltpu.VMEM((NQ, M // NQ, H * D), BF16),
            pltpu.VMEM((NQ, H * D // NQ, M), BF16),
            pltpu.VMEM((NBUF, H, T, D), BF16),
            pltpu.VMEM(((M + 1) * H // 2, D), U32),
            pltpu.VMEM(((DC + 1) * H // 2, D), U32),
            pltpu.VMEM((H * 8 + 8, D), F32),
            pltpu.VMEM((NJ, H, T), F32),
            pltpu.VMEM((NJ, H, T), F32),
            pltpu.VMEM((H, D), F32),
            pltpu.VMEM((H * 8 + 8, D), F32),
            pltpu.VMEM((DC // 128, H * 8 + 8, 128), F32),
            pltpu.VMEM((NA, H, AK), F32),
            pltpu.VMEM((NA, H, AK), BF16),
            pltpu.VMEM((H, DC), F32),
            pltpu.VMEM((DC // 128, H * 8 + 8, 128), F32),
            pltpu.VMEM((H * 8, D), F32),
            pltpu.VMEM((8, M), F32),
            pltpu.SemaphoreType.DMA((NBUF,)),
            pltpu.SemaphoreType.DMA((9,)),
            pltpu.SemaphoreType.DMA((2,)),
            pltpu.SemaphoreType.DMA((NTAIL,)),
        ],
        compiler_params=pltpu.CompilerParams(
            vmem_limit_bytes=80 * 1024 * 1024, disable_bounds_checks=True),
    )(A_x.reshape(B, M), A_c_kv.reshape(B, NQ, -1, DC), A_w_q.reshape(NQ, -1, D),
      A_w_uk.reshape(NQ, -1, D), A_w_uv.reshape(NQ, -1, D), A_w_o.reshape(NQ, -1, M),
      B_x.reshape(B, M), B_k_cache, B_v_cache, B_wq.reshape(NQ, -1, H * D), B_wo.reshape(NQ, -1, M))
    return out.reshape(B, 1, 2 * M)
```
